```python
import jax
import jax.numpy as jnp

def _softmax(x, axis=-1):
    return jax.nn.softmax(x, axis=axis)
def _gelu(x):
    return jax.nn.gelu(x, approximate=True)
def _silu(x):
    return jax.nn.silu(x)
def _sigmoid(x):
    return jax.nn.sigmoid(x)
def _layernorm(x, axis=-1, eps=1e-5):
    m = jnp.mean(x, axis=axis, keepdims=True)
    v = jnp.var(x, axis=axis, keepdims=True)
    return (x - m) / jnp.sqrt(v + eps)
def _scatter_add(tgt, idx, src, axis=0):
    return tgt.at[idx].add(src)
def _segment_sum(src, seg, n):
    return jax.ops.segment_sum(src, seg, n)
class _Rng:
    def __init__(self, key):
        self._k = key
    def _next(self):
        self._k, sub = jax.random.split(self._k)
        return sub
    def normal(self, shape):
        return jax.random.normal(self._next(), shape, dtype=jnp.bfloat16)
    def randint(self, lo, hi, shape):
        return jax.random.randint(self._next(), shape, lo, hi, dtype=jnp.int32)
    def uniform(self, shape, lo=0.0, hi=1.0):
        return jax.random.uniform(self._next(), shape, jnp.bfloat16, lo, hi)
    def permutation(self, n):
        return jax.random.permutation(self._next(), n)


kernel_name = 'standalone__layernorm_linear__prompt'

def setup_inputs():
    _rng = _Rng(jax.random.key(int.from_bytes(__import__("os").urandom(4), "little")))
    _w = (lambda a: (lambda t: t.astype(jnp.bfloat16) if jnp.issubdtype(t.dtype, jnp.floating) else t)(jnp.asarray(a)))
    B, S, D = 2, 2048, 1024
    return {
        "x": _w((lambda *s: _rng.normal(s) * 0.05)(B, S, D)),
        "g": _w((lambda *s: _rng.normal(s) * 0.05)(D) + 1.0),
        "b": _w((lambda *s: _rng.normal(s) * 0.05)(D)),
        "w": _w((lambda *s: _rng.normal(s) * 0.05)(D, D)),
    }

def reference(x, g, b, w):
    return (_layernorm(x, axis=-1) * g + b) @ w
```

```python
import jax
import jax.numpy as jnp
from jax import lax
import jax.experimental.pallas as pl
import jax.experimental.pallas.tpu as pltpu

EPS = 1e-5

R0 = 256
W_PIECES = 4
MID = 256
SUB = 128
NPIECE = 4
LOOP_ROWS = 512


def _layernorm(xb, g, b):
    x = xb.astype(jnp.float32)
    mean = jnp.mean(x, axis=-1, keepdims=True)
    xc = x - mean
    var = jnp.mean(xc * xc, axis=-1, keepdims=True)
    return (xc * lax.rsqrt(var + EPS) * g + b).astype(jnp.bfloat16)


def _make_kernel(M, D):
    n_loop = (M - R0 - MID) // LOOP_ROWS
    s_loop = LOOP_ROWS // SUB
    s_mid = MID // SUB
    ns0 = R0 // SUB
    kw = D // W_PIECES
    cw = D // NPIECE
    rw = SUB // NPIECE

    def kernel(x_hbm, g_hbm, b_hbm, w_hbm, o_hbm,
               x_v, w_v, o_v, g_v, b_v, y_buf, acc,
               sem_x, sem_w, sem_o, sem_gb, sem_fence):
        zero = pl.program_id(0)

        def x_copy(row, nrows, j):
            return pltpu.make_async_copy(
                x_hbm.at[pl.ds(row, nrows), :], x_v.at[pl.ds(row, nrows), :], sem_x.at[j])

        def fence():
            pl.semaphore_wait(sem_fence, 0)

        cp_g = pltpu.make_async_copy(g_hbm, g_v, sem_gb.at[0])
        cp_b = pltpu.make_async_copy(b_hbm, b_v, sem_gb.at[1])
        cp_x0 = x_copy(0, R0, 0)
        cp_xa = x_copy(R0, SUB, 1)
        cp_xm = x_copy(R0 + SUB, MID, 2)
        cp_w = [
            pltpu.make_async_copy(
                w_hbm.at[pl.ds(j * kw, kw), :], w_v.at[pl.ds(j * kw, kw), :], sem_w.at[j])
            for j in range(W_PIECES)
        ]
        cp_g.start()
        cp_b.start()
        cp_x0.start()
        fence()
        for c in cp_w:
            c.start()
            fence()
        cp_xa.start()
        fence()
        cp_xm.start()
        cp_g.wait()
        cp_b.wait()
        first = R0 + SUB + MID
        for i in range(n_loop):
            nrows = LOOP_ROWS if i < n_loop - 1 else LOOP_ROWS - SUB
            x_copy(first + i * LOOP_ROWS, nrows, 3 + i).start()
            fence()

        g = g_v[...].astype(jnp.float32).reshape(1, D)
        b = b_v[...].astype(jnp.float32).reshape(1, D)

        def ln_piece(x_row, slot, y_row):
            y_buf[slot, y_row:y_row + rw, :] = _layernorm(x_v[pl.ds(x_row, rw), :], g, b)

        def out_dma(row, nrows, col, ncols):
            pltpu.make_async_copy(
                o_v.at[pl.ds(row, nrows), pl.ds(col, ncols)],
                o_hbm.at[pl.ds(row, nrows), pl.ds(col, ncols)],
                sem_o,
            ).start(priority=1)

        cp_x0.wait()
        for s in range(ns0):
            for q in range(NPIECE):
                ln_piece(s * SUB + q * rw, s, q * rw)
        for j in range(W_PIECES):
            last = j == W_PIECES - 1
            cp_w[j].wait()
            if last:
                cp_xa.wait()
            for s in range(ns0):
                slot = s + zero if last else s
                p = jnp.dot(y_buf[slot, :, j * kw:(j + 1) * kw], w_v[j * kw:(j + 1) * kw, :],
                            preferred_element_type=jnp.float32)
                if j > 0:
                    p = p + acc[s]
                if not last:
                    acc[s] = p
                else:
                    o_v[s * SUB:(s + 1) * SUB, :] = p.astype(o_v.dtype)
                    per = NPIECE // ns0
                    for q in range(s * per, (s + 1) * per):
                        ln_piece(R0 + q * rw, ns0 + zero, q * rw)
        out_dma(0, R0, 0, D)

        def sub_block(row, next_row, parity):
            cur = ns0 + parity
            nxt = ns0 + 1 - parity
            for j in range(NPIECE):
                o_v[pl.ds(row, SUB), j * cw:(j + 1) * cw] = jnp.dot(
                    y_buf[cur], w_v[:, j * cw:(j + 1) * cw],
                    preferred_element_type=jnp.float32).astype(o_v.dtype)
                out_dma(row, SUB, j * cw, cw)
                ln_piece(next_row + j * rw, nxt, j * rw)

        cp_xm.wait()
        for s in range(s_mid):
            sub_block(R0 + s * SUB, R0 + (s + 1) * SUB, (s % 2) + zero)

        def body(i, carry):
            base = pl.multiple_of(R0 + MID + i * LOOP_ROWS, SUB)

            @pl.when(i < n_loop - 1)
            def _():
                x_copy(0, LOOP_ROWS, 3 + i).wait()

            @pl.when(i == n_loop - 1)
            def _():
                x_copy(0, LOOP_ROWS - SUB, 3 + i).wait()

            for s in range(s_loop):
                row = base + s * SUB
                if s + 1 < s_loop:
                    next_row = row + SUB
                else:
                    next_row = pl.multiple_of(jnp.minimum(row + SUB, M - SUB), SUB)
                sub_block(row, next_row, lax.rem(s_mid + i * s_loop + s, 2))
            return carry

        lax.fori_loop(0, n_loop, body, 0)
        pltpu.make_async_copy(o_v, o_hbm, sem_o).wait()

    return kernel, n_loop, ns0


@jax.jit
def pallas_standalone__layernorm_linear__prompt_kernel(
    x: jax.Array,
    g: jax.Array,
    b: jax.Array,
    w: jax.Array,
):
    B, S, D = x.shape
    M = B * S
    assert (M - R0 - MID) % LOOP_ROWS == 0 and D % (128 * NPIECE) == 0
    kernel, n_loop, ns0 = _make_kernel(M, D)
    any_spec = pl.BlockSpec(memory_space=pl.ANY)
    out = pl.pallas_call(
        kernel,
        grid=(1,),
        in_specs=[any_spec] * 4,
        out_specs=any_spec,
        out_shape=jax.ShapeDtypeStruct((M, D), x.dtype),
        scratch_shapes=[
            pltpu.VMEM((M, D), x.dtype),
            pltpu.VMEM((D, D), w.dtype),
            pltpu.VMEM((M, D), x.dtype),
            pltpu.VMEM((D,), g.dtype),
            pltpu.VMEM((D,), b.dtype),
            pltpu.VMEM((ns0 + 2, SUB, D), jnp.bfloat16),
            pltpu.VMEM((ns0, SUB, D), jnp.float32),
            pltpu.SemaphoreType.DMA((3 + n_loop,)),
            pltpu.SemaphoreType.DMA((W_PIECES,)),
            pltpu.SemaphoreType.DMA(()),
            pltpu.SemaphoreType.DMA((2,)),
            pltpu.SemaphoreType.REGULAR,
        ],
        compiler_params=pltpu.CompilerParams(vmem_limit_bytes=48 * 2**20),
    )(x.reshape(M, D), g, b, w)
    return out.reshape(B, S, D)
```

```python
import jax
import jax.numpy as jnp
from jax import lax
import jax.experimental.pallas as pl
import jax.experimental.pallas.tpu as pltpu

EPS = 1e-5

SUB = 128
NPIECE = 4
R0 = 256
W_PIECES = 4
MID = 256
LOOP_ROWS = 896


def _layernorm(xb, g, b):
    x = xb.astype(jnp.float32)
    mean = jnp.mean(x, axis=-1, keepdims=True)
    xc = x - mean
    var = jnp.mean(xc * xc, axis=-1, keepdims=True)
    return (xc * lax.rsqrt(var + EPS) * g + b).astype(jnp.bfloat16)


def _make_kernel(M, D):
    n_loop = (M - R0 - MID) // LOOP_ROWS
    s_loop = LOOP_ROWS // SUB
    s_mid = MID // SUB
    ns0 = R0 // SUB
    kw = D // W_PIECES
    cw = D // NPIECE
    rw = SUB // NPIECE
    first = R0 + MID + SUB

    def kernel(x_hbm, g_hbm, b_hbm, w_hbm, o_hbm,
               x_v, w_v, o_v, g_v, b_v, y_buf, acc,
               sem_x, sem_w, sem_o, sem_gb, sem_fence):
        zero = pl.program_id(0)

        def x_copy(row, nrows, j):
            return pltpu.make_async_copy(
                x_hbm.at[pl.ds(row, nrows), :], x_v.at[pl.ds(row, nrows), :], sem_x.at[j])

        def w_copy(j):
            k0 = j * kw if isinstance(j, int) else pl.multiple_of(j * kw, kw)
            return pltpu.make_async_copy(
                w_hbm.at[pl.ds(k0, kw), :], w_v.at[pl.ds(k0, kw), :], sem_w.at[j])

        def out_copy(row, nrows, col, ncols):
            return pltpu.make_async_copy(
                o_v.at[pl.ds(row, nrows), pl.ds(col, ncols)],
                o_hbm.at[pl.ds(row, nrows), pl.ds(col, ncols)],
                sem_o)

        def fence():
            pl.semaphore_signal(sem_fence, 1)
            pl.semaphore_wait(sem_fence, 1)

        cp_g = pltpu.make_async_copy(g_hbm, g_v, sem_gb.at[0])
        cp_b = pltpu.make_async_copy(b_hbm, b_v, sem_gb.at[1])
        cp_x0 = x_copy(0, R0, 0)
        cp_xa = x_copy(R0, SUB, 1)
        cp_xm = x_copy(R0 + SUB, MID, 2)
        cp_g.start()
        cp_b.start()
        cp_x0.start()
        fence()
        for j in range(W_PIECES):
            w_copy(j).start()
            fence()
        cp_xa.start()
        fence()
        cp_xm.start()
        cp_g.wait()
        cp_b.wait()
        for i in range(n_loop):
            nrows = LOOP_ROWS if i < n_loop - 1 else LOOP_ROWS - SUB
            x_copy(first + i * LOOP_ROWS, nrows, 3 + i).start()
            fence()

        g = g_v[...].astype(jnp.float32).reshape(1, D)
        b = b_v[...].astype(jnp.float32).reshape(1, D)

        def ln_piece(x_row, slot, y_row):
            y_buf[slot, y_row:y_row + rw, :] = _layernorm(x_v[pl.ds(x_row, rw), :], g, b)

        cp_x0.wait()
        for s in range(ns0):
            for q in range(NPIECE):
                ln_piece(s * SUB + q * rw, s, q * rw)
        for s in range(ns0):
            acc[s] = jnp.zeros((SUB, D), jnp.float32)

        def k_slice(j, carry):
            w_copy(j).wait()
            k0 = pl.multiple_of(j * kw, kw)
            for s in range(ns0):
                acc[s] = acc[s] + jnp.dot(
                    y_buf[s, :, pl.ds(k0, kw)], w_v[pl.ds(k0, kw), :],
                    preferred_element_type=jnp.float32)
            return carry

        lax.fori_loop(0, W_PIECES - 1, k_slice, 0)

        k0 = (W_PIECES - 1) * kw
        w_copy(W_PIECES - 1).wait()
        cp_xa.wait()
        for s in range(ns0):
            p = acc[s] + jnp.dot(y_buf[s + zero, :, k0:], w_v[k0:, :],
                                 preferred_element_type=jnp.float32)
            o_v[s * SUB:(s + 1) * SUB, :] = p.astype(o_v.dtype)
            for q in range(s * NPIECE // ns0, (s + 1) * NPIECE // ns0):
                ln_piece(R0 + q * rw, ns0 + zero, q * rw)

        def sub_block(row, next_row, parity, send):
            cur = ns0 + parity
            nxt = ns0 + 1 - parity
            for j in range(NPIECE):
                o_v[pl.ds(row, SUB), j * cw:(j + 1) * cw] = jnp.dot(
                    y_buf[cur], w_v[:, j * cw:(j + 1) * cw],
                    preferred_element_type=jnp.float32).astype(o_v.dtype)
                if send:
                    out_copy(row, SUB, j * cw, cw).start(priority=1)
                ln_piece(next_row + j * rw, nxt, j * rw)

        cp_xm.wait()
        for s in range(s_mid):
            sub_block(R0 + s * SUB, R0 + (s + 1) * SUB, (s % 2) + zero, send=False)

        def body(i, carry):
            base = pl.multiple_of(R0 + MID + i * LOOP_ROWS, SUB)

            @pl.when(i < n_loop - 1)
            def _():
                x_copy(pl.multiple_of(first + i * LOOP_ROWS, SUB), LOOP_ROWS, 3 + i).wait()

            @pl.when(i == n_loop - 1)
            def _():
                x_copy(M - LOOP_ROWS + SUB, LOOP_ROWS - SUB, 3 + i).wait()

            @pl.when(i == 0)
            def _():
                out_copy(0, R0 + MID, 0, D).start(priority=1)

            for s in range(s_loop):
                row = base + s * SUB
                if s + 1 < s_loop:
                    next_row = row + SUB
                else:
                    next_row = pl.multiple_of(jnp.minimum(row + SUB, M - SUB), SUB)
                sub_block(row, next_row, lax.rem(s_mid + i * s_loop + s, 2), send=True)
            return carry

        lax.fori_loop(0, n_loop, body, 0)
        out_copy(0, M, 0, D).wait()

    return kernel, n_loop, ns0


@jax.jit
def pallas_standalone__layernorm_linear__prompt_kernel(
    x: jax.Array,
    g: jax.Array,
    b: jax.Array,
    w: jax.Array,
):
    B, S, D = x.shape
    M = B * S
    assert (M - R0 - MID) % LOOP_ROWS == 0 and D % (128 * NPIECE) == 0
    kernel, n_loop, ns0 = _make_kernel(M, D)
    any_spec = pl.BlockSpec(memory_space=pl.ANY)
    out = pl.pallas_call(
        kernel,
        grid=(1,),
        in_specs=[any_spec] * 4,
        out_specs=any_spec,
        out_shape=jax.ShapeDtypeStruct((M, D), x.dtype),
        scratch_shapes=[
            pltpu.VMEM((M, D), x.dtype),
            pltpu.VMEM((D, D), w.dtype),
            pltpu.VMEM((M, D), x.dtype),
            pltpu.VMEM((D,), g.dtype),
            pltpu.VMEM((D,), b.dtype),
            pltpu.VMEM((ns0 + 2, SUB, D), jnp.bfloat16),
            pltpu.VMEM((ns0, SUB, D), jnp.float32),
            pltpu.SemaphoreType.DMA((3 + n_loop,)),
            pltpu.SemaphoreType.DMA((W_PIECES,)),
            pltpu.SemaphoreType.DMA(()),
            pltpu.SemaphoreType.DMA((2,)),
            pltpu.SemaphoreType.REGULAR,
        ],
        compiler_params=pltpu.CompilerParams(vmem_limit_bytes=48 * 2**20),
    )(x.reshape(M, D), g, b, w)
    return out.reshape(B, S, D)
```
